```python
import jax
import jax.numpy as jnp

def _softmax(x, axis=-1):
    return jax.nn.softmax(x, axis=axis)
def _gelu(x):
    return jax.nn.gelu(x, approximate=True)
def _silu(x):
    return jax.nn.silu(x)
def _sigmoid(x):
    return jax.nn.sigmoid(x)
def _layernorm(x, axis=-1, eps=1e-5):
    m = jnp.mean(x, axis=axis, keepdims=True)
    v = jnp.var(x, axis=axis, keepdims=True)
    return (x - m) / jnp.sqrt(v + eps)
def _scatter_add(tgt, idx, src, axis=0):
    return tgt.at[idx].add(src)
def _segment_sum(src, seg, n):
    return jax.ops.segment_sum(src, seg, n)
class _Rng:
    def __init__(self, key):
        self._k = key
    def _next(self):
        self._k, sub = jax.random.split(self._k)
        return sub
    def normal(self, shape):
        return jax.random.normal(self._next(), shape, dtype=jnp.bfloat16)
    def randint(self, lo, hi, shape):
        return jax.random.randint(self._next(), shape, lo, hi, dtype=jnp.int32)
    def uniform(self, shape, lo=0.0, hi=1.0):
        return jax.random.uniform(self._next(), shape, jnp.bfloat16, lo, hi)
    def permutation(self, n):
        return jax.random.permutation(self._next(), n)


kernel_name = 'standalone__gqa_block_cached__near_ridge'

def _fwd_setup_inputs():
    _rng = _Rng(jax.random.key(int.from_bytes(__import__("os").urandom(4), "little")))
    _w = (lambda a: (lambda t: t.astype(jnp.bfloat16) if jnp.issubdtype(t.dtype, jnp.floating) else t)(jnp.asarray(a)))
    B, Sq, D = 16, 64, 640
    Hq, Hkv, Sk, Dh = 32, 32, 512, 192
    assert Hq % Hkv == 0, (Hq, Hkv)
    return {
        "x": _w((lambda *s: _rng.normal(s) * 0.05)(B, Sq, D)),
        "k_cache": _w((lambda *s: _rng.normal(s) * 0.05)(B, Hkv, Sk, Dh)),
        "v_cache": _w((lambda *s: _rng.normal(s) * 0.05)(B, Hkv, Sk, Dh)),
        "wq": _w((lambda *s: _rng.normal(s) * 0.05)(D, Hq * Dh) * (D ** -0.5)),
        "wo": _w((lambda *s: _rng.normal(s) * 0.05)(Hq * Dh, D) * ((Hq * Dh) ** -0.5)),
    }

def _fwd_reference(x, k_cache, v_cache, wq, wo):
    B, Sq, D = x.shape
    Hq, Dh = 32, 192
    Hkv = k_cache.shape[1]
    rep = Hq // Hkv
    q = (lambda x, *d: x.transpose(*d))((x @ wq).reshape(B, Sq, Hq, Dh), 0, 2, 1, 3)
    k = jnp.repeat(k_cache, rep, axis=1)
    v = jnp.repeat(v_cache, rep, axis=1)
    scores = jnp.einsum("bhqd,bhkd->bhqk", q, k) * (Dh ** -0.5)
    p = _softmax(scores, axis=-1)
    o = jnp.einsum("bhqk,bhkd->bhqd", p, v)
    return (lambda x, *d: x.transpose(*d))(o, 0, 2, 1, 3).reshape(B, Sq, Hq * Dh) @ wo


def setup_inputs():
    _inp = _fwd_setup_inputs()
    _gk = jax.random.fold_in(jax.random.key(int.from_bytes(__import__("os").urandom(4), "little")), 2**31 - 1)
    _shapes = [[16, 64, 640]]
    _dtypes = ['bfloat16']
    _gks = jax.random.split(_gk, len(_shapes))
    _gs = [jax.random.normal(k, s, dtype=jnp.dtype(d)) * 0.05 for k, s, d in zip(_gks, _shapes, _dtypes)]
    _inp["grad_out"] = _gs[0]
    return _inp

def reference(x, k_cache, v_cache, wq, wo, grad_out):
    _const = dict()
    def _f(*_d):
        return _fwd_reference(**{'x': _d[0], 'k_cache': _d[1], 'v_cache': _d[2], 'wq': _d[3], 'wo': _d[4], **_const})
    _out, _vjp = jax.vjp(_f, x, k_cache, v_cache, wq, wo)
    _grads = _vjp(grad_out)
    _out0 = jnp.asarray(_out)
    return (_out0, *[jnp.asarray(_g) for _g in _grads])
```

```python
import functools

import jax
import jax.numpy as jnp
from jax import lax
import jax.experimental.pallas as pl
import jax.experimental.pallas.tpu as pltpu

F32, BF16 = jnp.float32, jnp.bfloat16
NN = (((1,), (0,)), ((), ()))
NT = (((1,), (1,)), ((), ()))
LOG2E = 1.4426950408889634

B, SQ, D, H, SK, DH = 16, 64, 640, 32, 512, 192
T = B * SQ
HP = H // 2
W = 2 * DH
SCALE = DH ** -0.5


def _dot(a, b, dims=NN):
    return lax.dot_general(a, b, dims, preferred_element_type=F32)


def _split_pair(z):
    za, zm, zb = z[:, :128], z[:, 128:256], z[:, 256:]
    lane = lax.broadcasted_iota(jnp.int32, zm.shape, 1)
    zero = jnp.zeros_like(zm)
    zm2 = jnp.concatenate([jnp.where(lane < 64, zm, zero), jnp.where(lane >= 64, zm, zero)], axis=0)
    return za, zm2, zb


def _scores(z, c_ref):
    za, zm, zb = _split_pair(z)
    s = jnp.concatenate([_dot(za, c_ref[0:128, :]), _dot(zb, c_ref[256:384, :])], axis=0) + _dot(zm, c_ref[128:256, :])
    zero = jnp.zeros_like(za)
    zt = jnp.concatenate([jnp.concatenate([za, zero], 0).T, zm.T, jnp.concatenate([zero, zb], 0).T], axis=0)
    return s, zt


def _softmax_fwd_bwd(s, dp):
    m = jnp.max(s, axis=1, keepdims=True)
    e = jnp.exp2((s - m) * (SCALE * LOG2E))
    p = e * (1.0 / jnp.sum(e, axis=1, keepdims=True))
    delta = jnp.sum(p * dp, axis=1, keepdims=True)
    ds = p * (dp - delta) * SCALE
    return p.astype(BF16), ds.astype(BF16)


def _apply(p, c_ref):
    a = _dot(p[:SQ], c_ref[0:128, :], NT)
    m = _dot(p, c_ref[128:256, :], NT)
    b = _dot(p[SQ:], c_ref[256:384, :], NT)
    lane = lax.broadcasted_iota(jnp.int32, a.shape, 1)
    return jnp.concatenate([a, jnp.where(lane < 64, m[:SQ], m[SQ:]), b], axis=1).astype(BF16)


def make_kernel(unroll=8, wrows=32, wb=8, rtail=1, wtail=1, no_dma=False, no_compute=False):
    def kernel(x_hbm, g_hbm, k_hbm, v_hbm, wq_hbm, wo_hbm,
               out_hbm, gx_hbm, dk_hbm, dv_hbm, gwq_hbm, gwo_hbm,
               x_s, g_s, xt_s, gt_s, q_s, do_s, o_s, dq_s, out_acc, gx_acc,
               wq_s, wo_s, k_s, v_s, gwq_s, gwo_s, dk_s, dv_s, sem, sem0):

        def cols(i):
            return pl.ds(pl.multiple_of(i * W, 128), W)

        def w_reads(i, slot):
            return [pltpu.make_async_copy(wq_hbm.at[:, cols(i)], wq_s.at[slot], sem.at[0, slot]),
                    pltpu.make_async_copy(wo_hbm.at[cols(i), :], wo_s.at[slot], sem.at[0, slot])]

        def kv_reads_main(i, slot):
            n = B - rtail
            return [pltpu.make_async_copy(k_hbm.at[:, i], k_s.at[slot], sem.at[0, slot]),
                    pltpu.make_async_copy(v_hbm.at[pl.ds(0, n), i], v_s.at[slot, pl.ds(0, n)], sem.at[0, slot])]

        def kv_reads_tail(i, slot):
            n = B - rtail
            return [pltpu.make_async_copy(v_hbm.at[pl.ds(n, rtail), i], v_s.at[slot, pl.ds(n, rtail)], sem.at[1, slot])]

        def kv_write(i, slot, s, b, r, sm):
            src, dst = ((dk_s, dk_hbm), (dv_s, dv_hbm))[s]
            return pltpu.make_async_copy(src.at[slot, pl.ds(b, wb), pl.ds(r, wrows)],
                                         dst.at[pl.ds(b, wb), i, pl.ds(r, wrows)], sem.at[sm, slot])

        pieces = [(s, b, r) for b in range(0, B, wb) for s in range(2) for r in range(0, W, wrows)]

        def w_writes(i, slot):
            return [pltpu.make_async_copy(gwq_s.at[slot], gwq_hbm.at[:, cols(i)], sem.at[2, slot]),
                    pltpu.make_async_copy(gwo_s.at[slot], gwo_hbm.at[cols(i), :], sem.at[2, slot])]

        def writes_main(i, slot):
            return w_writes(i, slot) + [kv_write(i, slot, *p, 2) for p in pieces[:len(pieces) - wtail]]

        def writes_tail(i, slot):
            return [kv_write(i, slot, *p, 3) for p in pieces[len(pieces) - wtail:]]

        def start(cs):
            if not no_dma:
                for c in cs:
                    c.start()

        def wait(cs):
            if not no_dma:
                for c in cs:
                    c.wait()

        cx = pltpu.make_async_copy(x_hbm, x_s, sem0.at[0])
        cg = pltpu.make_async_copy(g_hbm, g_s, sem0.at[1])
        cx.start()
        cg.start()
        start(w_reads(0, 0) + kv_reads_main(0, 0) + kv_reads_tail(0, 0))
        out_acc[...] = jnp.zeros_like(out_acc)
        gx_acc[...] = jnp.zeros_like(gx_acc)
        cx.wait()
        xt_s[...] = x_s[...].T
        cg.wait()
        gt_s[...] = g_s[...].T
        wait(w_reads(0, 0) + kv_reads_main(0, 0))

        def attention(slot, b0):
            pend = []

            def finish(b, rows, p, ds, qt, dt):
                dv_s[slot, b] = _dot(dt, p).astype(BF16)
                o_s[rows, :] = _apply(p, v_s.at[slot, b])
                dk_s[slot, b] = _dot(qt, ds).astype(BF16)
                dq_s[rows, :] = _apply(ds, k_s.at[slot, b])

            for j in range(unroll):
                b = b0 + j
                rows = pl.ds(pl.multiple_of(b * SQ, SQ), SQ)
                s, qt = _scores(q_s[rows, :], k_s.at[slot, b])
                dp, dt = _scores(do_s[rows, :], v_s.at[slot, b])
                p, ds = _softmax_fwd_bwd(s, dp)
                pend.append((b, rows, p, ds, qt, dt))
                if len(pend) > 1:
                    finish(*pend.pop(0))
            finish(*pend.pop(0))

        def step(i, _):
            slot = lax.rem(i, 2)
            if not no_compute:
                q_s[...] = _dot(x_s[...], wq_s[slot]).astype(BF16)
                do_s[...] = _dot(g_s[...], wo_s[slot], NT).astype(BF16)
            wait(kv_reads_tail(i, slot))

            def group(j, _):
                @pl.when(j * unroll == B // 2)
                def _():
                    @pl.when(i > 0)
                    def _():
                        wait(writes_main(i - 1, 1 - slot))

                    @pl.when(i + 1 < HP)
                    def _():
                        start(w_reads(i + 1, 1 - slot) + kv_reads_main(i + 1, 1 - slot) + kv_reads_tail(i + 1, 1 - slot))
                if not no_compute:
                    attention(slot, j * unroll)

            lax.fori_loop(0, B // unroll, group, None)

            if not no_compute:
                gwo_s[slot] = _dot(gt_s[...], o_s[...]).astype(BF16).T
                gwq_s[slot] = _dot(xt_s[...], dq_s[...]).astype(BF16)
                out_acc[...] += _dot(o_s[...], wo_s[slot])

            @pl.when(i > 0)
            def _():
                wait(writes_tail(i - 1, 1 - slot))

            @pl.when(i + 1 < HP)
            def _():
                wait(w_reads(i + 1, 1 - slot) + kv_reads_main(i + 1, 1 - slot))
            start(writes_main(i, slot) + writes_tail(i, slot))
            if not no_compute:
                gx_acc[...] += _dot(dq_s[...], wq_s[slot], NT)

        lax.fori_loop(0, HP, step, None)

        x_s[...] = out_acc[...].astype(BF16)
        co = pltpu.make_async_copy(x_s, out_hbm, sem0.at[0])
        co.start()
        g_s[...] = gx_acc[...].astype(BF16)
        cgx = pltpu.make_async_copy(g_s, gx_hbm, sem0.at[1])
        cgx.start()
        last = (HP - 1) % 2
        wait(writes_main(HP - 1, last) + writes_tail(HP - 1, last))
        co.wait()
        cgx.wait()

    return kernel


def build(**kw):
    @jax.jit
    def f(x, k_cache, v_cache, wq, wo, grad_out):
        kt = jnp.swapaxes(k_cache, 2, 3).reshape(B, HP, W, SK)
        vt = jnp.swapaxes(v_cache, 2, 3).reshape(B, HP, W, SK)
        sd = jax.ShapeDtypeStruct
        hbm = pl.BlockSpec(memory_space=pl.ANY)
        out, gx, dkt, dvt, gwq, gwo = pl.pallas_call(
            make_kernel(**kw),
            in_specs=[hbm] * 6,
            out_specs=[hbm] * 6,
            out_shape=[sd((T, D), BF16), sd((T, D), BF16), sd(kt.shape, BF16), sd(kt.shape, BF16),
                       sd(wq.shape, BF16), sd(wo.shape, BF16)],
            scratch_shapes=[
                pltpu.VMEM((T, D), BF16), pltpu.VMEM((T, D), BF16),
                pltpu.VMEM((D, T), BF16), pltpu.VMEM((D, T), BF16),
                pltpu.VMEM((T, W), BF16), pltpu.VMEM((T, W), BF16),
                pltpu.VMEM((T, W), BF16), pltpu.VMEM((T, W), BF16),
                pltpu.VMEM((T, D), F32), pltpu.VMEM((T, D), F32),
                pltpu.VMEM((2, D, W), BF16), pltpu.VMEM((2, W, D), BF16),
                pltpu.VMEM((2, B, W, SK), BF16), pltpu.VMEM((2, B, W, SK), BF16),
                pltpu.VMEM((2, D, W), BF16), pltpu.VMEM((2, W, D), BF16),
                pltpu.VMEM((2, B, W, SK), BF16), pltpu.VMEM((2, B, W, SK), BF16),
                pltpu.SemaphoreType.DMA((4, 2)), pltpu.SemaphoreType.DMA((2,)),
            ],
            compiler_params=pltpu.CompilerParams(vmem_limit_bytes=110 * 1024 * 1024),
        )(x.reshape(T, D), grad_out.reshape(T, D), kt, vt, wq, wo)
        unt = lambda a: jnp.swapaxes(a.reshape(B, H, DH, SK), 2, 3)
        return out.reshape(B, SQ, D), gx.reshape(B, SQ, D), unt(dkt), unt(dvt), gwq, gwo
    return f


_kernel = build()


@jax.jit
def pallas_standalone__gqa_block_cached__near_ridge_kernel(x, k_cache, v_cache, wq, wo, grad_out):
    return _kernel(x, k_cache, v_cache, wq, wo, grad_out)
```

```python
import contextlib

import jax
import jax.numpy as jnp
from jax import lax
import jax.experimental.pallas as pl
import jax.experimental.pallas.tpu as pltpu

F32, BF16 = jnp.float32, jnp.bfloat16
NN = (((1,), (0,)), ((), ()))
NT = (((1,), (1,)), ((), ()))
LOG2E = 1.4426950408889634

B, SQ, D, H, SK, DH = 16, 64, 640, 32, 512, 192
T = B * SQ
HP = H // 2
W = 2 * DH
SCALE = DH ** -0.5
U = B // 2
NS = 3
NW = 8
NG = 16
OS = 4
WG = ((0, 6), (6, 5), (11, 5), (6, 2), (8, 4), (12, 4), (0, 4), (4, 4))
PA, PB0, PB1, PC = range(4)


def _dot(a, b, dims=NN):
    return lax.dot_general(a, b, dims, preferred_element_type=F32)


def _softmax_fwd_bwd(s, dp):
    e = jnp.exp2(s - jnp.max(s, axis=1, keepdims=True))
    inv = 1.0 / jnp.sum(e, axis=1, keepdims=True)
    delta = jnp.sum(e * dp, axis=1, keepdims=True) * inv
    return (e * inv).astype(BF16), (e * (inv * (1.0 / LOG2E)) * (dp - delta)).astype(BF16)


def schedule(variant=0):
    def kv(j):
        return [('kv', j, 0), ('kv', j, 1)]

    def wr(j, gw=True, groups=(0, 1, 2)):
        out = [(a, j, g) for g in groups for a in ('dk', 'dv')]
        if gw is not None:
            jg = j if gw is True else gw
            out[3:3] = [('gwo', jg)]
            out[5:5] = [('gwq', jg)]
        return out

    s = {}
    s[-1, PC] = [('w', 0)] + kv(0) + [('w', 1), ('w', 2)] + kv(1) + [('w', 3)] + kv(2)
    s[0, PC] = [('w', 4)] + kv(3)
    s[1, PC] = [('w', 5)] + kv(4)
    for i in (2, 6, 10):
        a, b, c, d = (wr(j) for j in range(i - 2, i + 2))
        s[i, PB1] = ['sync'] + a[:5]
        s[i, PC] = a[5:] + b[:1]
        s[i + 1, PA] = b[1:5]
        s[i + 1, PB0] = b[5:]
        s[i + 1, PB1] = c[:5]
        s[i + 1, PC] = c[5:] + d[:1]
        s[i + 2, PA] = d[1:5]
        s[i + 2, PB0] = d[5:]
    for i in (4, 8):
        s[i, PB1] = ['sync', ('w', i + 2)] + kv(i + 1) + [('w', i + 3)] + kv(i + 2)
        s[i, PC] = [('w', i + 4)] + kv(i + 3)
        s[i + 1, PC] = [('w', i + 5)] + kv(i + 4)
    s[12, PB1] = wr(12, None, (6, 7))
    s[12, PC] = ['sync', ('w', 14)] + kv(13) + [('w', 15)] + kv(14) + kv(15)
    a, b, c = wr(12, True, (4, 5)), wr(13), wr(14)
    s[14, PB0] = ['sync'] + a + b[:1]
    s[14, PB1] = b[1:6]
    s[14, PC] = b[6:] + c[:2]
    s[15, PA] = c[2:5]
    s[15, PB0] = c[5:]
    s[15, PB1] = wr(15, None, (6, 7))
    s[15, PC] = wr(15, None, (4, 5))
    s[16, PA] = [('gwo', 15), ('gwq', 15)]
    late = [('gwq', 3), ('gwq', 7)]
    s = {p: [t for t in ts if t not in late] for p, ts in s.items()}
    s[15, PB1] += late
    return s


def plan(s):
    order = sorted(s)
    tails, prev = set(), None
    for p in order:
        for t in s[p]:
            if t == 'sync':
                tails.add(prev)
            else:
                prev = t

    def deadline(t):
        kind, j = t[:2]
        if kind == 'w':
            return j, PA
        if kind == 'kv':
            return j, PB0 + t[2]
        p = (j + NG, PC) if kind in ('gwo', 'gwq') else (j + NS, PB0 + (WG[t[2]][0] >= U))
        return min(p, (HP, PB0))

    ops = {}
    waits = {}
    for p in order:
        for t in s[p]:
            if t == 'sync':
                ops.setdefault(p, []).append(('wait', prev, 'main'))
                continue
            prev = t
            assert p < deadline(t), (p, t)
            if t in tails:
                ops.setdefault(p, []).extend([('start', t, 'main'), ('start', t, 'tail')])
                waits.setdefault(deadline(t), []).append(('wait', t, 'tail'))
            else:
                ops.setdefault(p, []).append(('start', t, 'all'))
                waits.setdefault(deadline(t), []).append(('wait', t, 'all'))
    for p in waits:
        ops.setdefault(p, []).extend(waits[p])
    return ops


NSEM = 6 + NW + 4 * NS


def make_kernel(pchunk=2, skew=2, cuts=tuple(range(24, W + 1, 40)), rtail=48, gwo_rows=40, orows=32, variant=0,
                tinb=True, scopes=False, no_dma=False, no_compute=False, patch=None):
    sched = schedule(variant)
    if patch:
        patch(sched)
    ops = plan(sched)
    chunks = [pl.ds(a, b - a) for a, b in zip((0,) + cuts, cuts)]

    def kernel(x_hbm, g_hbm, k_hbm, v_hbm, wq_hbm, wo_hbm,
               out_hbm, gx_hbm, dk_hbm, dv_hbm, gwq_hbm, gwo_hbm,
               x_s, g_s, xt_s, gt_s, q_s, do_s, qt_s, dot_s, p_s, o_s, dq_s, out_acc, gx_acc, out_s, gx_s,
               wq_s, wo_s, k_s, v_s, gwq_s, gwo_s, dk_s, dv_s, sem):

        def scope(n):
            return jax.named_scope('s_' + n) if scopes else contextlib.nullcontext()

        def pair(j):
            return pl.ds(pl.multiple_of(j * W, 128), W)

        def copies(op, kind, j, slot, arg, part):
            if kind == 'w':
                ws = j & (NW - 1)
                return [(wq_hbm.at[:, pair(j)], wq_s.at[ws], sem.at[6 + ws]), (wo_hbm.at[j], wo_s.at[ws], sem.at[6 + ws])]
            if kind == 'gwq':
                return [(gwq_s.at[j], gwq_hbm.at[:, pair(j)], sem.at[5])]
            if kind == 'gwo':
                rs = [pl.ds(r, min(gwo_rows, W - r)) for r in range(0, W, gwo_rows)] if op == 'start' else [pl.ds(0, W)]
                return [(gwo_s.at[j, r], gwo_hbm.at[j, r], sem.at[5]) for r in rs]
            base = 6 + NW + 4 * slot
            if kind == 'kv':
                bs = pl.ds(arg * U, U)
                sm = sem.at[2] if part == 'main' else sem.at[base + arg]
                rs = dict(all=pl.ds(0, W), main=pl.ds(0, W - rtail), tail=pl.ds(W - rtail, rtail))[part]
                return ([] if part == 'tail' else [(k_hbm.at[bs, j], k_s.at[slot, bs], sm)]) + \
                       [(v_hbm.at[bs, j, rs], v_s.at[slot, bs, rs], sm)]
            src, dst = (dk_s, dk_hbm) if kind == 'dk' else (dv_s, dv_hbm)
            bs = pl.ds(*WG[arg])
            sm = sem.at[3] if part == 'main' else sem.at[base + 2 + (WG[arg][0] >= U)]
            rs = dict(all=chunks, main=chunks[:-1], tail=chunks[-1:])[part]
            if op == 'wait':
                rs = [pl.ds(rs[0].start, sum(r.size for r in rs))]
            return [(src.at[slot, bs, r], dst.at[bs, j, r], sm) for r in rs]

        def run(todo, i, slots):
            if no_dma:
                return
            seq = []
            for op, (kind, dj, *arg), part in todo:
                cs = [(op, c) for c in copies(op, kind, i + dj, slots[dj % NS], arg[0] if arg else None, part)]
                if kind == 'gwo' and op == 'start' and len(seq) >= len(cs):
                    n = len(cs)
                    seq[-n:] = [c for both in zip(seq[-n:], cs) for c in both]
                else:
                    seq += cs
            for op, c in seq:
                c = pltpu.make_async_copy(*c)
                c.start() if op == 'start' else c.wait()

        def point(i, p, slots):
            cases = {}
            for j in range(HP):
                todo = tuple((op, (t[0], t[1] - j) + t[2:], part) for op, t, part in ops.get((j, p), ()))
                cut = max([n + 1 for n, o in enumerate(todo) if o[0] == 'start'], default=0)
                for key in [(0, todo[:cut])] + [(1, (o,)) for o in todo[cut:]]:
                    if key[1]:
                        cases[key] = cases.get(key, 0) | (1 << j)
            for (_, todo), mask in sorted(cases.items(), key=lambda kv: kv[0][0]):
                if mask == (1 << HP) - 1:
                    run(todo, i, slots)
                else:
                    pl.when((lax.shift_left(jnp.int32(1), i) & mask) != 0)(lambda: run(todo, i, slots))

        def wr_act(s, d, k):
            return [pltpu.make_async_copy(s.at[:, pl.ds(r, orows)], d.at[:, pl.ds(r, orows)], sem.at[k])
                    for r in range(0, T // OS, orows)]

        cx = pltpu.make_async_copy(x_hbm, x_s, sem.at[0])
        cg = pltpu.make_async_copy(g_hbm, g_s, sem.at[1])
        cx.start()
        cg.start()
        run(ops[-1, PC], 0, range(NS))
        out_acc[...] = jnp.zeros_like(out_acc)
        gx_acc[...] = jnp.zeros_like(gx_acc)
        cx.wait()
        xt_s[...] = x_s[...].T
        cg.wait()
        gt_s[...] = g_s[...].T

        def transposed(za, zm, zb):
            zero = jnp.zeros_like(za)
            return jnp.concatenate([jnp.concatenate([za, zero], 0).T, zm.T, jnp.concatenate([zero, zb], 0).T], axis=0)

        def project(src, w, dims, z_s, zt_s, scale):
            for c in range(0, B, pchunk):
                z = _dot(src[c * SQ:(c + pchunk) * SQ, :], w, dims)
                if scale is not None:
                    z = z * scale
                z = z.astype(BF16)
                for b in range(pchunk):
                    za, zm, zb = (z[b * SQ:(b + 1) * SQ, k:k + 128] for k in (0, 128, 256))
                    low = lax.broadcasted_iota(jnp.int32, zm.shape, 1) < 64
                    zero = jnp.zeros_like(zm)
                    zm = jnp.concatenate([jnp.where(low, zm, zero), jnp.where(low, zero, zm)], axis=0)
                    z_s[c + b] = jnp.concatenate([za, zm, zb], axis=0)
                    if not (tinb and zt_s is dot_s and c + pchunk == B):
                        zt_s[c + b] = transposed(za, zm, zb)

        def attention(slot, g):
            if tinb:
                for b in range(B - pchunk, B):
                    dot_s[b] = transposed(do_s[b, 0:64], do_s[b, 64:192], do_s[b, 192:256])
            for t in range(U + skew):
                j1, j2 = t, t - skew
                h1, h2 = j1 < U, j2 >= 0
                b1, b2 = g * U + j1, g * U + j2
                res = []
                for z_s, zt_s, c1_s, c2_s, r_s, dc_s, which in ((q_s, dot_s, k_s, v_s, o_s, dv_s, 0),
                                                                (do_s, qt_s, v_s, k_s, dq_s, dk_s, 1)):
                    if h1:
                        z = z_s.at[b1]
                        c1 = c1_s.at[slot, b1]
                    if h2:
                        p = p_s.at[j2 % (skew + 1), which]
                        c2 = c2_s.at[slot, b2]
                        dc_s[slot, b2] = _dot(zt_s[b2], p[...]).astype(BF16)
                        om = _dot(p[...], c2[128:256, :], NT)
                        oa = _dot(p[0:64, :], c2[0:128, :], NT)
                    if h1:
                        sa = _dot(z[0:64, :], c1[0:128, :])
                        sm = _dot(z[64:192, :], c1[128:256, :])
                    if h2:
                        ob = _dot(p[64:128, :], c2[256:384, :], NT)
                        low = lax.broadcasted_iota(jnp.int32, oa.shape, 1) < 64
                        r = jnp.concatenate([oa, jnp.where(low, om[:SQ], om[SQ:]), ob], axis=1)
                        if which == 1:
                            r = r * (SCALE * LOG2E)
                        r_s[pl.ds(pl.multiple_of(b2 * SQ, SQ), SQ), :] = r.astype(BF16)
                    if h1:
                        sb = _dot(z[192:256, :], c1[256:384, :])
                        res.append(jnp.concatenate([sa, sb], axis=0) + sm)
                if h1:
                    p_s[j1 % (skew + 1), 0], p_s[j1 % (skew + 1), 1] = _softmax_fwd_bwd(*res)

        def finish_acts():
            for a, b in zip(wr_act(out_s, out_hbm, 0), wr_act(gx_s, gx_hbm, 1)):
                a.start()
                b.start()

        def step(i, slots):
            ws = i & (NW - 1)
            with scope('PA'):
                point(i, PA, slots)
            if not no_compute:
                with scope('A'):
                    project(x_s, wq_s[ws], NN, q_s, qt_s, SCALE * LOG2E)
                    project(g_s, wo_s[ws], NT, do_s, dot_s, None)

            def group(g, _):
                with scope('PB'):
                    pl.when(g == 0)(lambda: point(i, PB0, slots))
                    pl.when(g == 1)(lambda: point(i, PB1, slots))
                if not no_compute:
                    with scope('B'):
                        attention(slots[0], g)

            lax.fori_loop(0, 2, group, None)

            with scope('PC'):
                point(i, PC, slots)

            if not no_compute:
                with scope('C'):
                    for acc, a_s, w, dims, dst, hbm, k in ((out_acc, o_s, wo_s, NN, out_s, out_hbm, 0),
                                                          (gx_acc, dq_s, wq_s, NT, gx_s, gx_hbm, 1)):
                        new = acc[...] + _dot(a_s[...], w[ws], dims)
                        acc[...] = new
                        dst[...] = new.astype(BF16).reshape(dst.shape)

                        @pl.when(i == HP - 1)
                        def _():
                            for c in wr_act(dst, hbm, k):
                                c.start()
                    gwo_s[i] = _dot(gt_s[...], o_s[...]).astype(BF16).T
                    gwq_s[i] = _dot(xt_s[...], dq_s[...]).astype(BF16)

            return slots[1:] + slots[:1]

        lax.fori_loop(0, HP, step, tuple(jnp.int32(k) for k in range(NS)))

        with scope('drain'):
            if no_compute:
                finish_acts()
            run(ops[HP, PA], 0, range(NS))
            run(ops[HP, PB0], 0, range(NS))
            pltpu.make_async_copy(out_s, out_hbm, sem.at[0]).wait()
            pltpu.make_async_copy(gx_s, gx_hbm, sem.at[1]).wait()

    return kernel


def build(checks=False, semchecks=True, flags=None, interpret=False, **kw):
    @jax.jit
    def f(x, k_cache, v_cache, wq, wo, grad_out):
        kt = jnp.swapaxes(k_cache, 2, 3).reshape(B, HP, W, SK)
        vt = jnp.swapaxes(v_cache, 2, 3).reshape(B, HP, W, SK)
        sd = jax.ShapeDtypeStruct
        hbm = pl.BlockSpec(memory_space=pl.ANY)
        act = (OS, T // OS, D)
        out, gx, dkt, dvt, gwq, gwo = pl.pallas_call(
            make_kernel(**kw),
            in_specs=[hbm] * 6,
            out_specs=[hbm] * 6,
            out_shape=[sd(act, BF16), sd(act, BF16), sd(kt.shape, BF16), sd(kt.shape, BF16),
                       sd(wq.shape, BF16), sd((HP, W, D), BF16)],
            scratch_shapes=[
                pltpu.VMEM((T, D), BF16), pltpu.VMEM((T, D), BF16),
                pltpu.VMEM((D, T), BF16), pltpu.VMEM((D, T), BF16),
                pltpu.VMEM((B, 256, 128), BF16), pltpu.VMEM((B, 256, 128), BF16),
                pltpu.VMEM((B, W, 128), BF16), pltpu.VMEM((B, W, 128), BF16),
                pltpu.VMEM((3, 2, 128, SK), BF16),
                pltpu.VMEM((T, W), BF16), pltpu.VMEM((T, W), BF16),
                pltpu.VMEM((T, D), F32), pltpu.VMEM((T, D), F32),
                pltpu.VMEM(act, BF16), pltpu.VMEM(act, BF16),
                pltpu.VMEM((NW, D, W), BF16), pltpu.VMEM((NW, W, D), BF16),
                pltpu.VMEM((NS, B, W, SK), BF16), pltpu.VMEM((NS, B, W, SK), BF16),
                pltpu.VMEM((NG, D, W), BF16), pltpu.VMEM((NG, W, D), BF16),
                pltpu.VMEM((NS, B, W, SK), BF16), pltpu.VMEM((NS, B, W, SK), BF16),
                pltpu.SemaphoreType.DMA((NSEM,)),
            ],
            compiler_params=pltpu.CompilerParams(vmem_limit_bytes=124 * 1024 * 1024, disable_bounds_checks=not checks, disable_semaphore_checks=not semchecks, flags=flags),
            interpret=interpret,
        )(x.reshape(T, D), grad_out.reshape(T, D), kt, vt, wq, wo.reshape(HP, W, D))
        unt = lambda a: jnp.swapaxes(a.reshape(B, H, DH, SK), 2, 3)
        return out.reshape(B, SQ, D), gx.reshape(B, SQ, D), unt(dkt), unt(dvt), gwq, gwo.reshape(wo.shape)
    return f


_kernel = build()


@jax.jit
def pallas_standalone__gqa_block_cached__near_ridge_kernel(x, k_cache, v_cache, wq, wo, grad_out):
    return _kernel(x, k_cache, v_cache, wq, wo, grad_out)
```

```python
import jax
import jax.numpy as jnp
from jax import lax
import jax.experimental.pallas as pl
import jax.experimental.pallas.tpu as pltpu

F32, BF16 = jnp.float32, jnp.bfloat16
NN = (((1,), (0,)), ((), ()))
NT = (((1,), (1,)), ((), ()))
LOG2E = 1.4426950408889634

B, SQ, D, H, SK, DH = 16, 64, 640, 32, 512, 192
T = B * SQ
HP = H // 2
W = 2 * DH
QSCALE = DH ** -0.5 * LOG2E
U = B // 2
SKEW = 2
PCHUNK = 2
NS = 7

GROUPS = ((0, 6), (6, 5), (11, 5), (0, 4), (4, 4), (8, 4), (12, 4))
WHOLE, LOW, HIGH = (0, 1, 2), (3, 4), (5, 6)
PIECES = ((0, 24),) + tuple((r, 40) for r in range(24, W, 40))
READ_TAIL = 48
ACT_SPLIT, ACT_ROWS = 4, 32

BEFORE_A, BEFORE_B0, BEFORE_B1, BEFORE_C = range(4)
START, FINISH, DRAIN = (-1, BEFORE_C), (HP, BEFORE_A), (HP, BEFORE_B0)

SEM_X, SEM_G, SEM_TURN_RD, SEM_TURN_WR, SEM_GW, SEM_W = range(6)
SEM_RING = SEM_W + HP
NUM_SEMS = SEM_RING + 4 * NS


def _schedule():
    def reads(steps, weights):
        kv = [[('kv', j, 0), ('kv', j, 1)] for j in steps]
        return [('w', weights[0])] + kv[0] + [('w', j) for j in weights[1:]] + sum(kv[1:], [])

    def writes(steps, groups):
        return [(a, j, g) for g in groups for a in ('dk', 'dv') for j in steps]

    def writes_of_two(j):
        o = writes((j, j + 1), WHOLE)
        return (o[:9] + [('gwo', j)] + o[9:10] + [('gwo', j + 1), ('gwq', j)]
                + o[10:11] + [('gwq', j + 1)] + o[11:])

    s = {}

    def spread(i, o):
        s[i, BEFORE_B0] += o[:1]
        s[i, BEFORE_B1], s[i, BEFORE_C] = o[1:4], o[4:8]
        s[i + 1, BEFORE_A], s[i + 1, BEFORE_B0] = o[8:13], o[13:]

    s[START] = reads(range(0, 7), range(0, 8))
    s[6, BEFORE_B1] = ['turn'] + reads(range(7, 13), range(8, 14))
    s[12, BEFORE_C] = ['turn'] + reads(range(13, 16), range(14, 16))
    for i in (3, 9):
        s[i, BEFORE_B0] = []
        for n in range(3):
            spread(i + n, writes_of_two(i - 3 + 2 * n))
        s[i, BEFORE_B1] = ['turn'] + s.pop((i, BEFORE_B0)) + s[i, BEFORE_B1]
    s[12, BEFORE_B1] = writes([12], LOW)
    high = writes([12], HIGH)
    s[14, BEFORE_B0] = ['turn'] + high[:2] + [('gwo', 12)] + high[2:] + [('gwq', 12)]
    spread(14, writes_of_two(13))
    s[15, BEFORE_B1] = writes([15], LOW)
    s[15, BEFORE_C] = writes([15], HIGH)
    s[FINISH] = [('gwq', 15), ('gwo', 15)]
    late = [('gwq', 1), ('gwq', 3)]
    s = {p: [t for t in ts if t not in late] for p, ts in s.items()}
    s[15, BEFORE_B1] += late
    return s


def _plan(sched):
    flat = [(p, t) for p in sorted(sched) for t in sched[p]]
    started_at = {t: p for p, t in flat}
    ops, waits = {}, []
    for n, (p, t) in enumerate(flat):
        todo = ops.setdefault(p, [])
        if t == 'turn':
            todo.append(('wait', flat[n - 1][1], 'main'))
        elif n + 1 < len(flat) and flat[n + 1][1] == 'turn':
            todo += [('start', t, 'main'), ('start', t, 'tail')]
            waits.append((p, t, 'tail'))
        else:
            todo.append(('start', t, 'all'))
            waits.append((p, t, 'all'))
    for p, t, part in waits:
        kind, j = t[:2]
        refill = None
        if kind == 'w':
            ready, due = START, (j, BEFORE_A)
        elif kind == 'kv':
            ready, due = START, (j, BEFORE_B0 + t[2])
        elif kind in ('gwq', 'gwo'):
            ready, due = (j + 1, BEFORE_A), DRAIN
        else:
            first, count = GROUPS[t[2]]
            ready = (j, BEFORE_B1 if first + count <= U else BEFORE_C)
            refill = ('kv', j + NS, first // U)
            due = started_at.get(refill, DRAIN)
        assert ready <= p < due, (t, ready, p, due)
        todo = ops.setdefault(due, [])
        at = [n for n, o in enumerate(todo) if o[:2] == ('start', refill)]
        todo.insert(at[0] if at else len(todo), ('wait', t, part))
    return ops


def _dot(a, b, dims=NN):
    return lax.dot_general(a, b, dims, preferred_element_type=F32)


def _low_lanes(shape):
    return lax.broadcasted_iota(jnp.int32, shape, 1) < 64


def _softmax_fwd_bwd(s, dp):
    e = jnp.exp2(s - jnp.max(s, axis=1, keepdims=True))
    inv = 1.0 / jnp.sum(e, axis=1, keepdims=True)
    delta = jnp.sum(e * dp, axis=1, keepdims=True) * inv
    return (e * inv).astype(BF16), (e * (inv * (1.0 / LOG2E)) * (dp - delta)).astype(BF16)


def _block_diag_t(za, zm, zb):
    zero = jnp.zeros_like(za)
    return jnp.concatenate([jnp.concatenate([za, zero], axis=0).T, zm.T,
                            jnp.concatenate([zero, zb], axis=0).T], axis=0)


def _kernel(x_hbm, g_hbm, k_hbm, v_hbm, wq_hbm, wo_hbm,
            out_hbm, gx_hbm, dk_hbm, dv_hbm, gwq_hbm, gwo_hbm,
            x_s, g_s, xt_s, gt_s, q_s, do_s, qt_s, dot_s, p_s, o_s, dq_s,
            out_acc, gx_acc, out_s, gx_s, wq_s, wo_s, k_s, v_s, sem):
    ops = _plan(_schedule())

    def copies(op, part, slot, kind, j, arg=None):
        pieces = dict(all=PIECES, main=PIECES[:-1], tail=PIECES[-1:])[part]
        if op == 'wait':
            pieces = [(pieces[0][0], sum(n for _, n in pieces))]
        if kind in ('w', 'gwq'):
            cols = pl.ds(pl.multiple_of(j * W, 128), W)
            if kind == 'gwq':
                return [(wq_s.at[j], gwq_hbm.at[:, cols], sem.at[SEM_GW])]
            return [(wq_hbm.at[:, cols], wq_s.at[j], sem.at[SEM_W + j]),
                    (wo_hbm.at[j], wo_s.at[j], sem.at[SEM_W + j])]
        if kind == 'gwo':
            return [(wo_s.at[j, pl.ds(*r)], gwo_hbm.at[j, pl.ds(*r)], sem.at[SEM_GW]) for r in pieces]
        ring = SEM_RING + 4 * slot
        if kind == 'kv':
            bs = pl.ds(arg * U, U)
            sm = sem.at[SEM_TURN_RD if part == 'main' else ring + arg]
            rows = pl.ds(*dict(all=(0, W), main=(0, W - READ_TAIL), tail=(W - READ_TAIL, READ_TAIL))[part])
            keys = [] if part == 'tail' else [(k_hbm.at[bs, j], k_s.at[slot, bs], sm)]
            return keys + [(v_hbm.at[bs, j, rows], v_s.at[slot, bs, rows], sm)]
        src, dst = (k_s, dk_hbm) if kind == 'dk' else (v_s, dv_hbm)
        bs = pl.ds(*GROUPS[arg])
        sm = sem.at[SEM_TURN_WR if part == 'main' else ring + 2 + GROUPS[arg][0] // U]
        return [(src.at[slot, bs, pl.ds(*r)], dst.at[bs, j, pl.ds(*r)], sm) for r in pieces]

    def run(todo, i, slots):
        seq = []
        for op, (kind, dj, *arg), part in todo:
            new = [(op, c) for c in copies(op, part, slots[dj % NS], kind, i + dj, *arg)]
            if (op, kind) == ('start', 'gwo') and len(seq) >= len(new):
                seq[-len(new):] = [c for both in zip(seq[-len(new):], new) for c in both]
            else:
                seq += new
        for op, c in seq:
            if op == 'start':
                pltpu.make_async_copy(*c).start()
            else:
                pltpu.make_async_copy(*c).wait()

    def transfers(i, place, slots):
        steps_of = {}
        for j in range(HP):
            todo = tuple((op, (t[0], t[1] - j) + t[2:], part) for op, t, part in ops.get((j, place), ()))
            cut = max([n + 1 for n, o in enumerate(todo) if o[0] == 'start'], default=0)
            for key in [(0, todo[:cut])] + [(1, (o,)) for o in todo[cut:]]:
                if key[1]:
                    steps_of[key] = steps_of.get(key, 0) | (1 << j)
        for (_, todo), mask in sorted(steps_of.items(), key=lambda item: item[0][0]):
            if mask == (1 << HP) - 1:
                run(todo, i, slots)
            else:
                pl.when((lax.shift_left(jnp.int32(1), i) & mask) != 0)(lambda: run(todo, i, slots))

    def project(src, w, dims, z_s, zt_s, scale=None):
        for c in range(0, B, PCHUNK):
            z = _dot(src[c * SQ:(c + PCHUNK) * SQ, :], w, dims)
            z = (z if scale is None else z * scale).astype(BF16)
            for b in range(PCHUNK):
                za, zm, zb = (z[b * SQ:(b + 1) * SQ, k:k + 128] for k in (0, 128, 256))
                low, zero = _low_lanes(zm.shape), jnp.zeros_like(zm)
                zm = jnp.concatenate([jnp.where(low, zm, zero), jnp.where(low, zero, zm)], axis=0)
                z_s[c + b] = jnp.concatenate([za, zm, zb], axis=0)
                if zt_s is qt_s or c + PCHUNK < B:
                    zt_s[c + b] = _block_diag_t(za, zm, zb)

    def attention(slot, half):
        for b in range(B - PCHUNK, B):
            dot_s[b] = _block_diag_t(do_s[b, 0:64], do_s[b, 64:192], do_s[b, 192:256])
        for n1 in range(U + SKEW):
            n2 = n1 - SKEW
            scores, outputs = n1 < U, n2 >= 0
            b1, b2 = half * U + n1, half * U + n2
            res = []
            for which, (z_s, c1_s, zt_s, c2_s, r_s) in enumerate(((q_s, k_s, dot_s, v_s, o_s),
                                                                  (do_s, v_s, qt_s, k_s, dq_s))):
                if scores:
                    z, c1 = z_s.at[b1], c1_s.at[slot, b1]
                if outputs:
                    p, c2 = p_s.at[n2 % (SKEW + 1), which], c2_s.at[slot, b2]
                    rm = _dot(p[...], c2[128:256, :], NT)
                    ra = _dot(p[0:64, :], c2[0:128, :], NT)
                if scores:
                    sa = _dot(z[0:64, :], c1[0:128, :])
                    sm = _dot(z[64:192, :], c1[128:256, :])
                if outputs:
                    rb = _dot(p[64:128, :], c2[256:384, :], NT)
                    r = jnp.concatenate([ra, jnp.where(_low_lanes(ra.shape), rm[:SQ], rm[SQ:]), rb], axis=1)
                    r_s[pl.ds(pl.multiple_of(b2 * SQ, SQ), SQ), :] = (r * QSCALE if which else r).astype(BF16)
                if scores:
                    sb = _dot(z[192:256, :], c1[256:384, :])
                    res.append(jnp.concatenate([sa, sb], axis=0) + sm)
                if outputs:
                    c2_s[slot, b2] = _dot(zt_s[b2], p[...]).astype(BF16)
            if scores:
                p_s[n1 % (SKEW + 1), 0], p_s[n1 % (SKEW + 1), 1] = _softmax_fwd_bwd(*res)

    def step(i, slots):
        transfers(i, BEFORE_A, slots)
        project(x_s, wq_s[i], NN, q_s, qt_s, QSCALE)
        project(g_s, wo_s[i], NT, do_s, dot_s)

        def half_of_b(half, _):
            pl.when(half == 0)(lambda: transfers(i, BEFORE_B0, slots))
            pl.when(half == 1)(lambda: transfers(i, BEFORE_B1, slots))
            attention(slots[0], half)

        lax.fori_loop(0, 2, half_of_b, None)

        transfers(i, BEFORE_C, slots)
        for acc, a_s, w_s, dims, res_s, res_hbm, k in ((out_acc, o_s, wo_s, NN, out_s, out_hbm, SEM_X),
                                                       (gx_acc, dq_s, wq_s, NT, gx_s, gx_hbm, SEM_G)):
            new = acc[...] + _dot(a_s[...], w_s[i], dims)
            acc[...] = new
            res_s[...] = new.astype(BF16).reshape(res_s.shape)

            @pl.when(i == HP - 1)
            def _():
                for r in range(0, T // ACT_SPLIT, ACT_ROWS):
                    rows = pl.ds(r, ACT_ROWS)
                    pltpu.make_async_copy(res_s.at[:, rows], res_hbm.at[:, rows], sem.at[k]).start()
        wo_s[i] = _dot(gt_s[...], o_s[...]).astype(BF16).T
        wq_s[i] = _dot(xt_s[...], dq_s[...]).astype(BF16)
        return slots[1:] + slots[:1]

    load_x = pltpu.make_async_copy(x_hbm, x_s, sem.at[SEM_X])
    load_g = pltpu.make_async_copy(g_hbm, g_s, sem.at[SEM_G])
    load_x.start()
    load_g.start()
    run(ops[START], 0, range(NS))
    out_acc[...] = jnp.zeros_like(out_acc)
    gx_acc[...] = jnp.zeros_like(gx_acc)
    load_x.wait()
    xt_s[...] = x_s[...].T
    load_g.wait()
    gt_s[...] = g_s[...].T

    lax.fori_loop(0, HP, step, tuple(jnp.int32(k) for k in range(NS)))

    run(ops[FINISH], 0, range(NS))
    run(ops[DRAIN], 0, range(NS))
    pltpu.make_async_copy(out_s, out_hbm, sem.at[SEM_X]).wait()
    pltpu.make_async_copy(gx_s, gx_hbm, sem.at[SEM_G]).wait()


@jax.jit
def pallas_standalone__gqa_block_cached__near_ridge_kernel(
    x: jax.Array,
    k_cache: jax.Array,
    v_cache: jax.Array,
    wq: jax.Array,
    wo: jax.Array,
    grad_out: jax.Array,
):
    cache = (B, HP, W, SK)
    act = (ACT_SPLIT, T // ACT_SPLIT, D)
    in_hbm = pl.BlockSpec(memory_space=pl.ANY)
    out, gx, dkt, dvt, gwq, gwo = pl.pallas_call(
        _kernel,
        in_specs=[in_hbm] * 6,
        out_specs=[in_hbm] * 6,
        out_shape=[jax.ShapeDtypeStruct(s, BF16) for s in (act, act, cache, cache, (D, HP * W), (HP, W, D))],
        scratch_shapes=(
            [pltpu.VMEM((T, D), BF16)] * 2
            + [pltpu.VMEM((D, T), BF16)] * 2
            + [pltpu.VMEM((B, 256, 128), BF16)] * 2
            + [pltpu.VMEM((B, W, 128), BF16)] * 2
            + [pltpu.VMEM((SKEW + 1, 2, 2 * SQ, SK), BF16)]
            + [pltpu.VMEM((T, W), BF16)] * 2
            + [pltpu.VMEM((T, D), F32)] * 2
            + [pltpu.VMEM(act, BF16)] * 2
            + [pltpu.VMEM((HP, D, W), BF16), pltpu.VMEM((HP, W, D), BF16)]
            + [pltpu.VMEM((NS, B, W, SK), BF16)] * 2
            + [pltpu.SemaphoreType.DMA((NUM_SEMS,))]
        ),
        compiler_params=pltpu.CompilerParams(
            vmem_limit_bytes=124 * 1024 * 1024,
            disable_bounds_checks=True,
            disable_semaphore_checks=True,
        ),
    )(
        x.reshape(T, D),
        grad_out.reshape(T, D),
        jnp.swapaxes(k_cache, 2, 3).reshape(cache),
        jnp.swapaxes(v_cache, 2, 3).reshape(cache),
        wq,
        wo.reshape(HP, W, D),
    )
    dk, dv = (jnp.swapaxes(a.reshape(B, H, DH, SK), 2, 3) for a in (dkt, dvt))
    return out.reshape(B, SQ, D), gx.reshape(B, SQ, D), dk, dv, gwq, gwo.reshape(H * DH, D)
```
